```python
import os as _os
_os.environ.setdefault("JAX_PLATFORMS", "cpu")
import jax
import jax.numpy as jnp

def _softmax(x, axis=-1):
    return jax.nn.softmax(x, axis=axis)
def _gelu(x):
    return jax.nn.gelu(x, approximate=True)
def _silu(x):
    return jax.nn.silu(x)
def _sigmoid(x):
    return jax.nn.sigmoid(x)
def _layernorm(x, axis=-1, eps=1e-5):
    m = jnp.mean(x, axis=axis, keepdims=True)
    v = jnp.var(x, axis=axis, keepdims=True)
    return (x - m) / jnp.sqrt(v + eps)
def _scatter_add(tgt, idx, src, axis=0):
    return tgt.at[idx].add(src)
def _segment_sum(src, seg, n):
    return jax.ops.segment_sum(src, seg, n)
class _Rng:
    def __init__(self, key):
        self._k = key
    def _next(self):
        self._k, sub = jax.random.split(self._k)
        return sub
    def normal(self, shape):
        return jax.random.normal(self._next(), shape, dtype=jnp.bfloat16)
    def randint(self, lo, hi, shape):
        return jax.random.randint(self._next(), shape, lo, hi, dtype=jnp.int32)
    def uniform(self, shape, lo=0.0, hi=1.0):
        return jax.random.uniform(self._next(), shape, jnp.bfloat16, lo, hi)
    def permutation(self, n):
        return jax.random.permutation(self._next(), n)


kernel_name = 'recurrent_scan__ssm_conv_s4__mixer_s_mlp__prompt'

def setup_inputs():
    _rng = _Rng(jax.random.key(int.from_bytes(__import__("os").urandom(4), "little")))
    _w = (lambda a: (lambda t: t.astype(jnp.bfloat16) if jnp.issubdtype(t.dtype, jnp.floating) else t)(jnp.asarray(a)))
    def _A_setup():
        B, L, D, N = 1, 2048, 512, 128
        A_re = -jnp.exp((lambda *s: _rng.normal(s) * 0.1)(D, N))
        A_im = jnp.pi * (lambda *s: _rng.normal(s) * 0.1)(D, N)
        B_re = (lambda *s: _rng.normal(s) * 0.1)(D, N)
        B_im = (lambda *s: _rng.normal(s) * 0.1)(D, N)
        C_re = (lambda *s: _rng.normal(s) * 0.1)(D, N)
        C_im = (lambda *s: _rng.normal(s) * 0.1)(D, N)
        log_dt = (lambda *s: _rng.normal(s) * 0.1)(D) * 0.5 - 4.0
        Dskip = (lambda *s: _rng.normal(s) * 0.05)(D)
        return {
            "u": _w((lambda *s: _rng.normal(s) * 0.05)(B, L, D)),
            "A_re": _w(A_re),
            "A_im": _w(A_im),
            "B_re": _w(B_re),
            "B_im": _w(B_im),
            "C_re": _w(C_re),
            "C_im": _w(C_im),
            "log_dt": _w(log_dt),
            "Dskip": _w(Dskip),
        }
    _A_in = _A_setup()

    def _B_setup():
        B, S, D, F = 1, 2048, 512, 1376
        return {
            "x":  _w((lambda *s: _rng.normal(s) * 0.05)(B, S, D)),
            "w1": _w((lambda *s: _rng.normal(s) * 0.8)(D, D) * (D ** -0.5)),
            "w2": _w((lambda *s: _rng.normal(s) * 0.8)(D, D) * (D ** -0.5)),
            "w3": _w((lambda *s: _rng.normal(s) * 0.8)(D, F) * (D ** -0.5)),
            "w4": _w((lambda *s: _rng.normal(s) * 0.8)(F, D) * (F ** -0.5)),
        }
    _B_in = _B_setup()

    return {
        "A_u": _A_in["u"],
        "A_A_re": _A_in["A_re"],
        "A_A_im": _A_in["A_im"],
        "A_B_re": _A_in["B_re"],
        "A_B_im": _A_in["B_im"],
        "A_C_re": _A_in["C_re"],
        "A_C_im": _A_in["C_im"],
        "A_log_dt": _A_in["log_dt"],
        "A_Dskip": _A_in["Dskip"],
        "B_x": _B_in["x"],
        "B_w1": _B_in["w1"],
        "B_w2": _B_in["w2"],
        "B_w3": _B_in["w3"],
        "B_w4": _B_in["w4"],
    }

def reference(A_u, A_A_re, A_A_im, A_B_re, A_B_im, A_C_re, A_C_im, A_log_dt, A_Dskip, B_x, B_w1, B_w2, B_w3, B_w4):
    def _A_ref(u, A_re, A_im, B_re, B_im, C_re, C_im, log_dt, Dskip):
        Bsz, L, D = u.shape
        dt = jnp.exp(log_dt)[:, None]
        A = A_re + 1j * A_im
        Bc = B_re + 1j * B_im
        Cc = C_re + 1j * C_im
        logdA = dt * A
        dB = dt * Bc
        l = (lambda x, dt: x.astype(dt))(jnp.arange(L), A_re.dtype)
        P = jnp.exp(logdA[:, :, None] * l[None, None, :])
        K = jnp.einsum("dn,dnl,dn->dl", Cc, P, dB).real
        L2 = 2 * L
        Kp = jnp.pad(K, ((0, 0), (0, L)))
        up = (lambda x, *d: x.transpose(*d))(u, 0, 2, 1)
        up = jnp.pad(up, ((0, 0), (0, 0), (0, L)))
        Kf = (lambda x, axes=(-2,-1): jnp.fft.rfft2(x.astype(jnp.float32), axes=axes))(Kp[:, None, :], axes=(-2, -1))
        Uf = (lambda x, axes=(-2,-1): jnp.fft.rfft2(x.astype(jnp.float32), axes=axes))(up[:, :, None, :], axes=(-2, -1))
        Yf = Uf * Kf[None, :, :, :]
        y = (lambda x, s, axes=(-2,-1): jnp.fft.irfft2(x, s=s, axes=axes).astype(jnp.bfloat16))(Yf, (1, L2), axes=(-2, -1))[:, :, 0, :L]
        y = (lambda x, *d: x.transpose(*d))(y, 0, 2, 1) + u * Dskip[None, None, :]
        return y

    def _B_ref(x, w1, w2, w3, w4):
        B, S, D = x.shape
        h = _gelu(_layernorm(x, axis=-1) @ w1)
        c = D // 4
        g0 = jnp.pad(h[:, :, 0*c:1*c], ((0, 0), (1, 0), (0, 0)))[:, :S, :]
        g1 = jnp.pad(h[:, :, 1*c:2*c], ((0, 0), (0, 1), (0, 0)))[:, 1:, :]
        g2 = jnp.pad(h[:, :, 2*c:3*c], ((0, 0), (2, 0), (0, 0)))[:, :S, :]
        g3 = jnp.pad(h[:, :, 3*c:   ], ((0, 0), (0, 2), (0, 0)))[:, 2:, :]
        hs = jnp.concatenate([g0, g1, g2, g3], axis=-1) @ w2
        x1 = x + hs
        h2 = _gelu(_layernorm(x1, axis=-1) @ w3) @ w4
        return x1 + h2

    x = A_u
    xn = _layernorm(x, axis=-1)
    s = _A_ref(xn, A_A_re, A_A_im, A_B_re, A_B_im, A_C_re, A_C_im, A_log_dt, A_Dskip)
    g = _silu(_B_ref(xn, B_w1, B_w2, B_w3, B_w4))
    return x + s * g
```

```python
import functools
import operator
import numpy as np
import jax
import jax.numpy as jnp
from jax import lax
import jax.experimental.pallas as pl
import jax.experimental.pallas.tpu as pltpu

L, D, N, F = 2048, 512, 128, 1376
Q = 128
NCH = L // Q
TM = 256
NT = L // TM
EPS = 1e-5
F32, BF16 = jnp.float32, jnp.bfloat16

YS = [0, 1, 2, 3, 4, 5, 6, 7, 256, 258, 260, 262, 512, 516, 768, 772,
      1024, 1280, 1536, 1792, 2048]
NY = 24
NX = 32
ST = 65
DP = 8 * ST
PITCH = DP + 1


def _round_bf16_int(v):
    u = np.asarray(v, np.float32).view(np.uint32).astype(np.uint64)
    u = (u + 0x7FFF + ((u >> 16) & 1)) & 0xFFFF0000
    return u.astype(np.uint32).view(np.float32).astype(np.int64)


def _constants():
    f = np.concatenate([np.arange(0, Q, 2), np.arange(1, Q, 2)])
    th = 2.0 * np.pi * (f + 0.5) / (2 * Q)
    t = np.arange(Q)
    fwd = np.concatenate([np.cos(th[:, None] * t), -np.sin(th[:, None] * t)], 0)
    ang = th[None, :] * (Q + t)[:, None]
    inv = np.concatenate([np.cos(ang), -np.sin(ang)], 1) * (2.0 / (2 * Q))
    lr = _round_bf16_int(np.arange(L))
    pieces, fk = [], np.zeros((NCH, 2 * Q, Q))
    for j in range(NCH):
        pj = []
        for l0 in range(Q):
            l = int(lr[j * Q + l0])
            yi = max(i for i, y in enumerate(YS) if y <= l and (l - y) % 8 == 0 and l - y < 8 * NX)
            x = (l - YS[yi]) // 8
            key = (yi, x // 8)
            if key not in pj:
                pj.append(key)
            fk[j, :, pj.index(key) * 8 + x % 8] += fwd[:, l0]
        assert len(pj) <= 16
        pieces.append(pj)
    return fwd, inv, fk, pieces


_FWD, _INV, _FK, _PIECES = _constants()


def _gelu(x):
    c = 0.7978845608028654
    return (0.5 * x) * (1.0 + jnp.tanh(x * (c + (c * 0.044715) * (x * x))))


def _cmul(a, b):
    return a[0] * b[0] - a[1] * b[1], a[0] * b[1] + a[1] * b[0]


def _csq(a):
    return a[0] * a[0] - a[1] * a[1], 2.0 * (a[0] * a[1])


def _dot(a, b):
    return jnp.dot(a, b, preferred_element_type=F32)


def _kernel(u_h, are_h, aim_h, bre_h, bim_h, cre_h, cim_h, ldt_ref, dsk_ref,
            w1_h, w2_h, w3_h, w4_h, fwd_h, inv_h, fk_h,
            o_h,
            u_v, p_v, w1_v, w2_v, w3_v, w4_v, fwd_v, inv_v, fk_v,
            dt_v, q_v, wt_v, vt_v, kg_v, ks_v, kf_v, uf_v, up_v, z_v, h_v, g_v, o_v, xn_v,
            sem, osem):
    pars = (are_h, aim_h, bre_h, bim_h, cre_h, cim_h)
    cp_p = [pltpu.make_async_copy(pars[i], p_v.at[i], sem.at[i]) for i in range(6)]
    big = ((fk_h, fk_v), (fwd_h, fwd_v), (u_h, u_v), (w1_h, w1_v), (w2_h, w2_v),
           (w3_h, w3_v), (w4_h, w4_v), (inv_h, inv_v))
    cp_b = [pltpu.make_async_copy(s, d, sem.at[6 + i]) for i, (s, d) in enumerate(big)]
    for c in cp_p:
        c.start()

    dt_row = jnp.exp(ldt_ref[...].astype(F32)).astype(BF16).astype(F32).reshape(1, D)
    for b in range(4):
        dt_v[b * 128:(b + 1) * 128, :] = jnp.broadcast_to(dt_row[:, b * 128:(b + 1) * 128], (128, 128)).T
    dt_v[D:DP, :] = jnp.zeros((DP - D, N), F32)
    for c in cp_p:
        c.wait()
    for c in cp_b:
        c.start()
    for k in range(6):
        q_v[k, 0:D, :] = p_v[k].astype(F32)
        q_v[k, D:DP, :] = jnp.zeros((DP - D, N), F32)

    def tab(i):
        tr = lambda k: pl.ds(k * PITCH + i, 8, stride=ST)
        dt = dt_v[tr(0), :]
        ld = lambda k: q_v[k, tr(0), :]
        ar, ai = dt * ld(0), dt * ld(1)
        e = jnp.exp(ar)
        p1 = (e * jnp.cos(ai), e * jnp.sin(ai))
        c0 = _cmul((ld(4), ld(5)), (dt * ld(2), dt * ld(3)))
        w = {0: c0}
        for k in range(1, 8):
            w[k] = _cmul(w[k - 1], p1)
        p8 = _csq(_csq(_csq(p1)))
        v = p8
        vt_v[0, tr(0), :] = jnp.ones((8, N), F32)
        vt_v[1, tr(0), :] = jnp.zeros((8, N), F32)
        for x in range(1, NX):
            vt_v[0, tr(x), :] = v[0]
            vt_v[1, tr(x), :] = v[1]
            v = _cmul(v, p8)
        p256 = v
        w[256] = _cmul(w[0], p256)
        for k in (2, 4, 6):
            w[256 + k] = _cmul(w[k], p256)
        w[512], w[516] = _cmul(w[256], p256), _cmul(w[260], p256)
        w[768], w[772] = _cmul(w[512], p256), _cmul(w[516], p256)
        for k in range(1024, 2049, 256):
            w[k] = _cmul(w[k - 256], p256)
        for yi, y in enumerate(YS):
            wt_v[0, tr(yi), :] = w[y][0]
            wt_v[1, tr(yi), :] = -w[y][1]
        for yi in range(len(YS), NY):
            wt_v[0, tr(yi), :] = jnp.zeros((8, N), F32)
            wt_v[1, tr(yi), :] = jnp.zeros((8, N), F32)
    h_v[0:8, :] = jnp.zeros((8, D), F32)
    h_v[L + 8:L + 16, :] = jnp.zeros((8, D), F32)
    up_v[...] = jnp.zeros((2 * Q, D), F32)
    def pha(i):
        r0 = pl.multiple_of(i * TM, TM)
        x = u_v[pl.ds(r0, TM), :].astype(F32)
        m = jnp.mean(x, axis=-1, keepdims=True)
        xc = x - m
        v = jnp.mean(xc * xc, axis=-1, keepdims=True)
        rs = lax.rsqrt(v + EPS)
        xn = xc * rs
        xnb = xn.astype(BF16)
        xn_v[pl.ds(r0, TM), :] = xnb
        ln2 = (xn * lax.rsqrt(v * rs * rs + EPS)).astype(BF16)
        h_v[pl.ds(r0 + 8, TM), :] = _gelu(_dot(ln2, w1_v[...]))
        prev = up_v[...]
        for c in range(TM // Q):
            uf = _dot(fwd_v[...], xnb[c * Q:(c + 1) * Q, :])
            ch = i * (TM // Q) + c
            uf_v[ch, 0:64, :] = prev[0:64] + uf[128:192]
            uf_v[ch, 64:128, :] = prev[64:128] - uf[192:256]
            uf_v[ch, 128:192, :] = prev[128:192] - uf[0:64]
            uf_v[ch, 192:256, :] = prev[192:256] + uf[64:128]
            prev = uf
        up_v[...] = prev
    def mlp(i):
        r0 = pl.multiple_of(i * TM, TM)
        hs = jnp.concatenate([
            h_v[pl.ds(r0, TM + 16), k * 128:(k + 1) * 128][o:o + TM]
            for k, o in enumerate((7, 9, 6, 10))], 1).astype(BF16)
        xn = xn_v[pl.ds(r0, TM), :].astype(F32)
        x1 = xn + _dot(hs, w2_v[...])
        m = jnp.mean(x1, axis=-1, keepdims=True)
        xc = x1 - m
        v = jnp.mean(xc * xc, axis=-1, keepdims=True)
        ln = (xc * lax.rsqrt(v + EPS)).astype(BF16)
        a = _gelu(lax.dot_general(ln, w3_v[...], (((1,), (1,)), ((), ())), preferred_element_type=F32))
        z = x1 + _dot(a.astype(BF16), w4_v[...])
        g_v[pl.ds(r0, TM), :] = z * (0.5 + 0.5 * jnp.tanh(0.5 * z))
    def mac(p):
        rr = pl.ds(pl.multiple_of((p // 4) * 16, 16), 16)
        ri = pl.ds(pl.multiple_of((p // 4) * 16 + Q, 16), 16)
        cc = pl.ds(pl.multiple_of((p % 4) * 128, 128), 128)
        us = [uf_v[m, rr, cc] + uf_v[m, ri, cc] for m in range(NCH)]
        ks = [kf_v[m, rr, cc] + kf_v[m, ri, cc] for m in range(NCH)]
        kd = [kf_v[m, ri, cc] - kf_v[m, rr, cc] for m in range(NCH)]
        add = lambda ts: functools.reduce(operator.add, ts)
        for m in range(NCH):
            js = range(m + 1)
            s1 = add([kf_v[j, rr, cc] * us[m - j] for j in js])
            z_v[m, ri, cc] = (s1 + add([kd[j] * uf_v[m - j, rr, cc] for j in js])).astype(BF16)
            z_v[m, rr, cc] = (s1 - add([ks[j] * uf_v[m - j, ri, cc] for j in js])).astype(BF16)

    dsk = dsk_ref[...].astype(F32).reshape(1, D)
    def out_cp(i):
        rows = pl.ds(pl.multiple_of(i * TM, TM), TM)
        return pltpu.make_async_copy(o_v.at[rows], o_h.at[rows], osem.at[i])
    def fin(i):
        r0 = pl.multiple_of(i * TM, TM)
        x, xn = u_v[pl.ds(r0, TM), :].astype(F32), xn_v[pl.ds(r0, TM), :].astype(F32)
        y = jnp.concatenate([_dot(inv_v[...], z_v[i * (TM // Q) + c]) for c in range(TM // Q)], 0)
        s = y + xn * dsk
        o_v[pl.ds(r0, TM), :] = (x + s * g_v[pl.ds(r0, TM), :]).astype(BF16)
        out_cp(i).start()
    tab(ST - 1)
    for c in cp_b[1:4]:
        c.wait()
    with jax.named_scope("phaseA"):
        def l1(i, _):
            pha(i)
            for k in range(8):
                tab(i * 8 + k)
        lax.fori_loop(0, NT, l1, None)
    lane = lax.broadcasted_iota(jnp.int32, (NY, 128), 1)

    with jax.named_scope("kgen"):
        def kgen(g, _):
            def gather(t2, n):
                return jnp.concatenate(
                    [jnp.concatenate([t2[ri, pl.ds(g + 128 * dd, n, stride=PITCH), :] for dd in range(4)], 0).astype(BF16)
                     for ri in range(2)], 1)
            wg = gather(wt_v, NY)
            vg = gather(vt_v, NX)
            o = lax.dot_general(wg, vg, (((1,), (1,)), ((), ())), preferred_element_type=F32)
            c = o[0:NY]
            for dd in range(1, 4):
                c = jnp.where(lane >= 32 * dd, o[NY * dd:NY * (dd + 1)], c)
            kg_v[pl.ds(g, NY, stride=129), :] = c
        lax.fori_loop(0, 128, kgen, None, unroll=8)

    with jax.named_scope("krelayout"):
        for yi in range(len(YS)):
            m = kg_v[yi * 129:yi * 129 + 128, :].T
            for j in range(NCH):
                for pi, (py, xb) in enumerate(_PIECES[j]):
                    if py == yi:
                        for dd in range(4):
                            ks_v[j, pi * 8:(pi + 1) * 8, dd * 128:(dd + 1) * 128] = (
                                m[dd * 32 + xb * 8:dd * 32 + xb * 8 + 8, :])
        for j in range(NCH):
            n = len(_PIECES[j])
            if n < 16:
                ks_v[j, n * 8:, :] = jnp.zeros((Q - n * 8, D), F32)

    cp_b[0].wait()
    with jax.named_scope("kdft"):
        def kdft(j, _):
            kf_v[j] = _dot(fk_v[j], ks_v[j].astype(BF16))
        lax.fori_loop(0, NCH, kdft, None, unroll=4)

    for c in cp_b[4:]:
        c.wait()
    lax.fori_loop(0, 32, lambda i, _: mac(i), None)
    lax.fori_loop(0, NT, lambda i, _: mlp(i), None)
    lax.fori_loop(0, NT, lambda i, _: fin(i), None)
    for i in range(NT):
        out_cp(i).wait()


@jax.jit
def pallas_recurrent_scan__ssm_conv_s4__mixer_s_mlp__prompt_kernel(
    A_u: jax.Array,
    A_A_re: jax.Array,
    A_A_im: jax.Array,
    A_B_re: jax.Array,
    A_B_im: jax.Array,
    A_C_re: jax.Array,
    A_C_im: jax.Array,
    A_log_dt: jax.Array,
    A_Dskip: jax.Array,
    B_x: jax.Array,
    B_w1: jax.Array,
    B_w2: jax.Array,
    B_w3: jax.Array,
    B_w4: jax.Array,
):
    hbm = pl.BlockSpec(memory_space=pltpu.HBM)
    vm = pl.BlockSpec(memory_space=pltpu.VMEM)
    scratch = [
        pltpu.VMEM((L, D), BF16),
        pltpu.VMEM((6, D, N), BF16),
        pltpu.VMEM((D, D), BF16), pltpu.VMEM((D, D), BF16),
        pltpu.VMEM((F, D), BF16), pltpu.VMEM((F, D), BF16),
        pltpu.VMEM((2 * Q, Q), BF16), pltpu.VMEM((Q, 2 * Q), BF16), pltpu.VMEM((NCH, 2 * Q, Q), BF16),
        pltpu.VMEM((DP, N), F32),
        pltpu.VMEM((6, DP, N), F32),
        pltpu.VMEM((2, NY * PITCH, N), F32),
        pltpu.VMEM((2, NX * PITCH, N), F32),
        pltpu.VMEM((129 * NY, 128), F32),
        pltpu.VMEM((NCH, Q, D), F32),
        pltpu.VMEM((NCH, 2 * Q, D), F32),
        pltpu.VMEM((NCH, 2 * Q, D), F32),
        pltpu.VMEM((2 * Q, D), F32),
        pltpu.VMEM((NCH, 2 * Q, D), BF16),
        pltpu.VMEM((L + 16, D), F32),
        pltpu.VMEM((L, D), F32),
        pltpu.VMEM((L, D), BF16),
        pltpu.VMEM((L, D), BF16),
        pltpu.SemaphoreType.DMA((14,)),
        pltpu.SemaphoreType.DMA((NT,)),
    ]
    out = pl.pallas_call(
        _kernel,
        out_shape=jax.ShapeDtypeStruct((L, D), BF16),
        in_specs=[hbm] * 7 + [vm, vm] + [hbm] * 7,
        out_specs=hbm,
        scratch_shapes=scratch,
        compiler_params=pltpu.CompilerParams(vmem_limit_bytes=110 * 1024 * 1024),
    )(A_u.reshape(L, D), A_A_re, A_A_im, A_B_re, A_B_im, A_C_re, A_C_im,
      A_log_dt, A_Dskip, B_w1, B_w2, B_w3.T, B_w4,
      _FWD.astype(BF16), _INV.astype(BF16), _FK.astype(BF16))
    return out.reshape(1, L, D)
```
